```python
import os as _os
_os.environ.setdefault("JAX_PLATFORMS", "cpu")
import jax
import jax.numpy as jnp

def _softmax(x, axis=-1):
    return jax.nn.softmax(x, axis=axis)
def _gelu(x):
    return jax.nn.gelu(x, approximate=True)
def _silu(x):
    return jax.nn.silu(x)
def _sigmoid(x):
    return jax.nn.sigmoid(x)
def _layernorm(x, axis=-1, eps=1e-5):
    m = jnp.mean(x, axis=axis, keepdims=True)
    v = jnp.var(x, axis=axis, keepdims=True)
    return (x - m) / jnp.sqrt(v + eps)
def _scatter_add(tgt, idx, src, axis=0):
    return tgt.at[idx].add(src)
def _segment_sum(src, seg, n):
    return jax.ops.segment_sum(src, seg, n)
class _Rng:
    def __init__(self, key):
        self._k = key
    def _next(self):
        self._k, sub = jax.random.split(self._k)
        return sub
    def normal(self, shape):
        return jax.random.normal(self._next(), shape, dtype=jnp.bfloat16)
    def randint(self, lo, hi, shape):
        return jax.random.randint(self._next(), shape, lo, hi, dtype=jnp.int32)
    def uniform(self, shape, lo=0.0, hi=1.0):
        return jax.random.uniform(self._next(), shape, jnp.bfloat16, lo, hi)
    def permutation(self, n):
        return jax.random.permutation(self._next(), n)


kernel_name = 'parallel_sum__ssm_conv_s4__mixer_channel_mlp__prompt'

def setup_inputs():
    _rng = _Rng(jax.random.key(int.from_bytes(__import__("os").urandom(4), "little")))
    _w = (lambda a: (lambda t: t.astype(jnp.bfloat16) if jnp.issubdtype(t.dtype, jnp.floating) else t)(jnp.asarray(a)))
    def _A_setup():
        B, L, D, N = 1, 2048, 512, 128
        A_re = -jnp.exp((lambda *s: _rng.normal(s) * 0.1)(D, N))
        A_im = jnp.pi * (lambda *s: _rng.normal(s) * 0.1)(D, N)
        B_re = (lambda *s: _rng.normal(s) * 0.1)(D, N)
        B_im = (lambda *s: _rng.normal(s) * 0.1)(D, N)
        C_re = (lambda *s: _rng.normal(s) * 0.1)(D, N)
        C_im = (lambda *s: _rng.normal(s) * 0.1)(D, N)
        log_dt = (lambda *s: _rng.normal(s) * 0.1)(D) * 0.5 - 4.0
        Dskip = (lambda *s: _rng.normal(s) * 0.05)(D)
        return {
            "u": _w((lambda *s: _rng.normal(s) * 0.05)(B, L, D)),
            "A_re": _w(A_re),
            "A_im": _w(A_im),
            "B_re": _w(B_re),
            "B_im": _w(B_im),
            "C_re": _w(C_re),
            "C_im": _w(C_im),
            "log_dt": _w(log_dt),
            "Dskip": _w(Dskip),
        }
    _A_in = _A_setup()

    def _B_setup():
        B, S, D, F = 1, 2048, 512, 1792
        return {
            "x": _w((lambda *s: _rng.normal(s) * 0.05)(B, S, D)),
            "w1": _w((lambda *s: _rng.normal(s) * 0.2)(D, F) * (D ** -0.5)),
            "b1": _w((lambda *s: _rng.normal(s) * 0.2)(F)),
            "w2": _w((lambda *s: _rng.normal(s) * 0.2)(F, D) * (F ** -0.5)),
            "b2": _w((lambda *s: _rng.normal(s) * 0.05)(D)),
        }
    _B_in = _B_setup()

    return {
        "A_u": _A_in["u"],
        "A_A_re": _A_in["A_re"],
        "A_A_im": _A_in["A_im"],
        "A_B_re": _A_in["B_re"],
        "A_B_im": _A_in["B_im"],
        "A_C_re": _A_in["C_re"],
        "A_C_im": _A_in["C_im"],
        "A_log_dt": _A_in["log_dt"],
        "A_Dskip": _A_in["Dskip"],
        "B_x": _B_in["x"],
        "B_w1": _B_in["w1"],
        "B_b1": _B_in["b1"],
        "B_w2": _B_in["w2"],
        "B_b2": _B_in["b2"],
    }

def reference(A_u, A_A_re, A_A_im, A_B_re, A_B_im, A_C_re, A_C_im, A_log_dt, A_Dskip, B_x, B_w1, B_b1, B_w2, B_b2):
    def _A_ref(u, A_re, A_im, B_re, B_im, C_re, C_im, log_dt, Dskip):
        Bsz, L, D = u.shape
        dt = jnp.exp(log_dt)[:, None]
        A = A_re + 1j * A_im
        Bc = B_re + 1j * B_im
        Cc = C_re + 1j * C_im
        logdA = dt * A
        dB = dt * Bc
        l = (lambda x, dt: x.astype(dt))(jnp.arange(L), A_re.dtype)
        P = jnp.exp(logdA[:, :, None] * l[None, None, :])
        K = jnp.einsum("dn,dnl,dn->dl", Cc, P, dB).real
        L2 = 2 * L
        Kp = jnp.pad(K, ((0, 0), (0, L)))
        up = (lambda x, *d: x.transpose(*d))(u, 0, 2, 1)
        up = jnp.pad(up, ((0, 0), (0, 0), (0, L)))
        Kf = (lambda x, axes=(-2,-1): jnp.fft.rfft2(x.astype(jnp.float32), axes=axes))(Kp[:, None, :], axes=(-2, -1))
        Uf = (lambda x, axes=(-2,-1): jnp.fft.rfft2(x.astype(jnp.float32), axes=axes))(up[:, :, None, :], axes=(-2, -1))
        Yf = Uf * Kf[None, :, :, :]
        y = (lambda x, s, axes=(-2,-1): jnp.fft.irfft2(x, s=s, axes=axes).astype(jnp.bfloat16))(Yf, (1, L2), axes=(-2, -1))[:, :, 0, :L]
        y = (lambda x, *d: x.transpose(*d))(y, 0, 2, 1) + u * Dskip[None, None, :]
        return y

    def _B_ref(x, w1, b1, w2, b2):
        y = _layernorm(x, axis=-1)
        h = _gelu(jnp.einsum("bsd,df->bsf", y, w1) + b1)
        return jnp.einsum("bsf,fd->bsd", h, w2) + b2

    x = A_u
    xn = _layernorm(x, axis=-1)
    return x + _A_ref(xn, A_A_re, A_A_im, A_B_re, A_B_im, A_C_re, A_C_im, A_log_dt, A_Dskip) + _B_ref(xn, B_w1, B_b1, B_w2, B_b2)
```

```python
import functools
import math

import jax
import jax.numpy as jnp
import numpy as np
from jax import lax
import jax.experimental.pallas as pl
import jax.experimental.pallas.tpu as pltpu

_S = 128


def _bf16_round_np(x):
    u = np.asarray(x, np.float32).view(np.uint32).astype(np.uint64)
    u = (u + 0x7FFF + ((u >> 16) & 1)) & 0xFFFF0000
    return u.astype(np.uint32).view(np.float32)


@functools.lru_cache(maxsize=None)
def _const_tables(L):
    S = _S
    C = L // S
    n = np.arange(S)
    b = np.arange(S)
    ang = np.pi * (2 * b[:, None] + 1) * n[None, :] / (2 * S)
    fwd_t = np.concatenate([np.cos(ang), -np.sin(ang)], axis=0)
    q = _bf16_round_np(np.arange(L)).astype(np.int64)
    fwdk_t = np.zeros((C, 2 * S, S))
    xcol = np.zeros((C, 2 * S, 1))
    for j in range(C):
        for i in range(S):
            src = q[S * j + i] - S * j
            if src < S:
                fwdk_t[j, :, src] += fwd_t[:, i]
            else:
                assert src == S
                xcol[j, :, 0] += fwd_t[:, i]
    n2 = np.arange(2 * S)
    ang2 = np.pi * (2 * b[None, :] + 1) * n2[:, None] / (2 * S)
    inv = np.concatenate([np.cos(ang2) / S, -np.sin(ang2) / S], axis=1)
    return fwd_t, fwdk_t, xcol, inv


def _cmul(ar, ai, br, bi):
    return ar * br - ai * bi, ar * bi + ai * br


def _gelu_tanh(h):
    c = math.sqrt(2.0 / math.pi)
    return 0.5 * h * (1.0 + jnp.tanh(c * (h + 0.044715 * (h * h * h))))


def _kernel(x_ref, are_ref, aim_ref, bre_ref, bim_ref, cre_ref, cim_ref, ldt_ref, dsk_ref,
            w1_ref, b1_ref, w2_ref, b2_ref, fwd_ref, fwdk_ref, xcol_ref, inv_ref,
            o_ref,
            xn_s, y2_s, pw_s, g_s, gt_s, uf_s, kf_s, yf_s, yacc_s,
            *, L, D, N, F, TB):
    S = _S
    C = L // S
    f32 = jnp.float32
    bf16 = jnp.bfloat16

    def ln(v):
        m = jnp.mean(v, axis=-1, keepdims=True)
        c = v - m
        var = jnp.mean(c * c, axis=-1, keepdims=True)
        return c * lax.rsqrt(var + 1e-5)

    def ln_body(i, _):
        r0 = pl.multiple_of(i * TB, TB)
        xv = x_ref[pl.ds(r0, TB), :].astype(f32)
        xn = ln(xv).astype(bf16)
        xn_s[pl.ds(r0, TB), :] = xn
        y2_s[pl.ds(r0, TB), :] = ln(xn.astype(f32)).astype(bf16)
        return 0

    lax.fori_loop(0, L // TB, ln_body, 0)

    dt = jnp.exp(ldt_ref[...].astype(f32)).astype(bf16).astype(f32)
    lr = dt * are_ref[...].astype(f32)
    li = dt * aim_ref[...].astype(f32)
    mag = jnp.exp(lr)
    zr, zi = mag * jnp.cos(li), mag * jnp.sin(li)
    for k in range(7):
        pw_s[k] = zr
        pw_s[7 + k] = zi
        if k < 6:
            zr, zi = _cmul(zr, zi, zr, zi)
    mag = jnp.exp(lr * float(S))
    er, ei = mag * jnp.cos(li * float(S)), mag * jnp.sin(li * float(S))
    for k in range(5):
        pw_s[14 + k] = er
        pw_s[19 + k] = ei
        if k < 4:
            er, ei = _cmul(er, ei, er, ei)
    cbr, cbi = _cmul(cre_ref[...].astype(f32), cim_ref[...].astype(f32),
                     dt * bre_ref[...].astype(f32), dt * bim_ref[...].astype(f32))
    pw_s[24] = cbr
    pw_s[25] = cbi

    sub = lax.broadcasted_iota(jnp.int32, (8, N), 0)
    one = jnp.ones((8, N), f32)
    zero = jnp.zeros((8, N), f32)

    def powtab(d, rbase, ibase, nrows):
        def row(k, base):
            return pw_s[base + k, pl.ds(d, 1), :]
        pr = jnp.where((sub & 1) == 1, row(0, rbase), one)
        pi = jnp.where((sub & 1) == 1, row(0, ibase), zero)
        for k in (1, 2):
            tr = jnp.where((sub & (1 << k)) != 0, row(k, rbase), one)
            ti = jnp.where((sub & (1 << k)) != 0, row(k, ibase), zero)
            pr, pi = _cmul(pr, pi, tr, ti)
        k = 3
        n = 8
        while n < nrows:
            qr, qi = _cmul(pr, pi, row(k, rbase), row(k, ibase))
            pr = jnp.concatenate([pr, qr], axis=0)
            pi = jnp.concatenate([pi, qi], axis=0)
            n *= 2
            k += 1
        return pr, pi

    def split(v):
        h = v.astype(bf16)
        return h, (v - h.astype(f32)).astype(bf16)

    dn_nt = (((1,), (1,)), ((), ()))

    def g_body(d, _):
        pr, pi = powtab(d, 0, 7, S)
        ar, ai = powtab(d, 14, 19, 32)
        ar, ai = _cmul(ar, ai, pw_s[24, pl.ds(d, 1), :], pw_s[25, pl.ds(d, 1), :])
        lhs = jnp.concatenate([ar[:24], -ai[:24]], axis=1)
        rhs = jnp.concatenate([pr, pi], axis=1)
        lh, ll = split(lhs)
        rh, rl = split(rhs)
        g = lax.dot_general(lh, rh, dn_nt, preferred_element_type=f32)
        g = g + lax.dot_general(ll, rh, dn_nt, preferred_element_type=f32)
        g = g + lax.dot_general(lh, rl, dn_nt, preferred_element_type=f32)
        g_s[d] = g
        return 0

    lax.fori_loop(0, D, g_body, 0, unroll=2)

    for r in range(C + 1):
        gt_s[r] = g_s[:, r, :].T

    for c in range(C):
        uf_s[c] = jnp.dot(fwd_ref[...], xn_s[pl.ds(c * S, S), :], preferred_element_type=f32)
        kf = jnp.dot(fwdk_ref[c], gt_s[c].astype(bf16), preferred_element_type=f32)
        kf_s[c] = kf + xcol_ref[c] * gt_s[c + 1, pl.ds(0, 1), :]

    def t1_body(t1, _):
        for cb in range(D // 128):
            cs = pl.ds(cb * 128, 128)

            def j_body(j, acc):
                yr, yi = acc
                ur = uf_s[t1 - j, pl.ds(0, S), cs]
                ui = uf_s[t1 - j, pl.ds(S, S), cs]
                kr = kf_s[j, pl.ds(0, S), cs]
                ki = kf_s[j, pl.ds(S, S), cs]
                return yr + (ur * kr - ui * ki), yi + (ur * ki + ui * kr)

            z0 = jnp.zeros((S, 128), f32)
            yr, yi = lax.fori_loop(0, t1 + 1, j_body, (z0, z0))
            yf_s[t1, pl.ds(0, S), cs] = yr.astype(bf16)
            yf_s[t1, pl.ds(S, S), cs] = yi.astype(bf16)
        return 0

    lax.fori_loop(0, C, t1_body, 0)

    for c in range(C):
        o = jnp.dot(inv_ref[...], yf_s[c], preferred_element_type=f32)
        if c == 0:
            yacc_s[0] = o[:S]
        else:
            yacc_s[c] = yacc_s[c] + o[:S]
        yacc_s[c + 1] = o[S:]

    def mlp_body(i, _):
        r0 = pl.multiple_of(i * TB, TB)
        h = jnp.dot(y2_s[pl.ds(r0, TB), :], w1_ref[...], preferred_element_type=f32)
        h = h + b1_ref[...].astype(f32)
        gl = _gelu_tanh(h).astype(bf16)
        mlp = jnp.dot(gl, w2_ref[...], preferred_element_type=f32) + b2_ref[...].astype(f32)
        nb = TB // S
        yc = jnp.concatenate([yacc_s[i * nb + k] for k in range(nb)], axis=0)
        xn = xn_s[pl.ds(r0, TB), :].astype(f32)
        a_branch = yc.astype(bf16).astype(f32) + xn * dsk_ref[...].astype(f32)
        out = x_ref[pl.ds(r0, TB), :].astype(f32) + a_branch + mlp
        o_ref[pl.ds(r0, TB), :] = out.astype(o_ref.dtype)
        return 0

    lax.fori_loop(0, L // TB, mlp_body, 0)


@jax.jit
def pallas_parallel_sum__ssm_conv_s4__mixer_channel_mlp__prompt_kernel(
    A_u: jax.Array,
    A_A_re: jax.Array,
    A_A_im: jax.Array,
    A_B_re: jax.Array,
    A_B_im: jax.Array,
    A_C_re: jax.Array,
    A_C_im: jax.Array,
    A_log_dt: jax.Array,
    A_Dskip: jax.Array,
    B_x: jax.Array,
    B_w1: jax.Array,
    B_b1: jax.Array,
    B_w2: jax.Array,
    B_b2: jax.Array,
):
    del B_x
    Bsz, L, D = A_u.shape
    assert Bsz == 1
    N = A_A_re.shape[1]
    F = B_w1.shape[1]
    S = _S
    C = L // S
    TB = 256
    fwd_t, fwdk_t, xcol, inv = _const_tables(L)
    bf16 = jnp.bfloat16
    consts = (
        jnp.asarray(fwd_t, bf16),
        jnp.asarray(fwdk_t, bf16),
        jnp.asarray(xcol, jnp.float32),
        jnp.asarray(inv, bf16),
    )
    f32 = jnp.float32
    scratch = [
        pltpu.VMEM((L, D), bf16),
        pltpu.VMEM((L, D), bf16),
        pltpu.VMEM((26, D, N), f32),
        pltpu.VMEM((D, 24, S), f32),
        pltpu.VMEM((C + 1, S, D), f32),
        pltpu.VMEM((C, 2 * S, D), f32),
        pltpu.VMEM((C, 2 * S, D), f32),
        pltpu.VMEM((C, 2 * S, D), bf16),
        pltpu.VMEM((C + 1, S, D), f32),
    ]
    out = pl.pallas_call(
        functools.partial(_kernel, L=L, D=D, N=N, F=F, TB=TB),
        out_shape=jax.ShapeDtypeStruct((L, D), A_u.dtype),
        scratch_shapes=scratch,
        compiler_params=pltpu.CompilerParams(vmem_limit_bytes=110 * 1024 * 1024),
    )(
        A_u.reshape(L, D),
        A_A_re, A_A_im, A_B_re, A_B_im, A_C_re, A_C_im,
        A_log_dt.reshape(D, 1),
        A_Dskip.reshape(1, D),
        B_w1, B_b1.reshape(1, F), B_w2, B_b2.reshape(1, D),
        *consts,
    )
    return out.reshape(Bsz, L, D)
```

```python
import functools
import math

import jax
import jax.numpy as jnp
import numpy as np
from jax import lax
import jax.experimental.pallas as pl
import jax.experimental.pallas.tpu as pltpu

_S = 128


def _bf16_round_np(x):
    u = np.asarray(x, np.float32).view(np.uint32).astype(np.uint64)
    u = (u + 0x7FFF + ((u >> 16) & 1)) & 0xFFFF0000
    return u.astype(np.uint32).view(np.float32)


@functools.lru_cache(maxsize=None)
def _const_tables(L):
    S = _S
    C = L // S
    n = np.arange(S)
    b = np.arange(S)
    ang = np.pi * (2 * b[:, None] + 1) * n[None, :] / (2 * S)
    fwd_t = np.concatenate([np.cos(ang), -np.sin(ang)], axis=0)
    q = _bf16_round_np(np.arange(L)).astype(np.int64)
    fwdk_t = np.zeros((C, 2 * S, S))
    xcol = np.zeros((C, 2 * S, 1))
    for j in range(C):
        for i in range(S):
            src = q[S * j + i] - S * j
            if src < S:
                fwdk_t[j, :, src] += fwd_t[:, i]
            else:
                assert src == S
                xcol[j, :, 0] += fwd_t[:, i]
    n2 = np.arange(2 * S)
    ang2 = np.pi * (2 * b[None, :] + 1) * n2[:, None] / (2 * S)
    inv = np.concatenate([np.cos(ang2) / S, -np.sin(ang2) / S], axis=1)
    return fwd_t, fwdk_t, xcol, inv


def _cmul(ar, ai, br, bi):
    return ar * br - ai * bi, ar * bi + ai * br


def _gelu_tanh(h):
    c = math.sqrt(2.0 / math.pi)
    return 0.5 * h * (1.0 + jnp.tanh(c * (h + 0.044715 * (h * h * h))))


def _kernel(x_ref, are_ref, aim_ref, bre_ref, bim_ref, cre_ref, cim_ref, ldt_ref, dsk_ref,
            w1_ref, b1_ref, w2_ref, b2_ref, fwd_ref, fwdk_ref, xcol_ref, inv_ref,
            o_ref,
            xn_s, y2_s, pw_s, g_s, gt_s, uf_s, kf_s, yf_s, yacc_s, w1_s, w2_s, sem,
            *, L, D, N, F, TB):
    S = _S
    C = L // S
    f32 = jnp.float32
    bf16 = jnp.bfloat16

    w1_copy = pltpu.make_async_copy(w1_ref, w1_s, sem.at[0])
    w2_copy = pltpu.make_async_copy(w2_ref, w2_s, sem.at[1])
    w1_copy.start()
    w2_copy.start()

    def ln(v):
        m = jnp.mean(v, axis=-1, keepdims=True)
        c = v - m
        var = jnp.mean(c * c, axis=-1, keepdims=True)
        return c * lax.rsqrt(var + 1e-5)

    def ln_body(i, _):
        r0 = pl.multiple_of(i * TB, TB)
        xv = x_ref[pl.ds(r0, TB), :].astype(f32)
        xn = ln(xv).astype(bf16)
        xn_s[pl.ds(r0, TB), :] = xn
        y2_s[pl.ds(r0, TB), :] = ln(xn.astype(f32)).astype(bf16)
        return 0

    lax.fori_loop(0, L // TB, ln_body, 0)

    dt = jnp.exp(ldt_ref[...].astype(f32)).astype(bf16).astype(f32)
    lr = dt * are_ref[...].astype(f32)
    li = dt * aim_ref[...].astype(f32)
    mag = jnp.exp(lr)
    zr, zi = mag * jnp.cos(li), mag * jnp.sin(li)
    for k in range(7):
        pw_s[k] = zr
        pw_s[7 + k] = zi
        if k < 6:
            zr, zi = _cmul(zr, zi, zr, zi)
    mag = jnp.exp(lr * float(S))
    er, ei = mag * jnp.cos(li * float(S)), mag * jnp.sin(li * float(S))
    for k in range(5):
        pw_s[14 + k] = er
        pw_s[19 + k] = ei
        if k < 4:
            er, ei = _cmul(er, ei, er, ei)
    cbr, cbi = _cmul(cre_ref[...].astype(f32), cim_ref[...].astype(f32),
                     dt * bre_ref[...].astype(f32), dt * bim_ref[...].astype(f32))
    pw_s[24] = cbr
    pw_s[25] = cbi

    sub = lax.broadcasted_iota(jnp.int32, (8, N), 0)
    one = jnp.ones((8, N), f32)
    zero = jnp.zeros((8, N), f32)

    def powtab(d, rbase, ibase, nrows):
        def row(k, base):
            return pw_s[base + k, pl.ds(d, 1), :]
        pr = jnp.where((sub & 1) == 1, row(0, rbase), one)
        pi = jnp.where((sub & 1) == 1, row(0, ibase), zero)
        for k in (1, 2):
            tr = jnp.where((sub & (1 << k)) != 0, row(k, rbase), one)
            ti = jnp.where((sub & (1 << k)) != 0, row(k, ibase), zero)
            pr, pi = _cmul(pr, pi, tr, ti)
        k = 3
        n = 8
        while n < nrows:
            qr, qi = _cmul(pr, pi, row(k, rbase), row(k, ibase))
            pr = jnp.concatenate([pr, qr], axis=0)
            pi = jnp.concatenate([pi, qi], axis=0)
            n *= 2
            k += 1
        return pr, pi

    def split(v):
        h = v.astype(bf16)
        return h, (v - h.astype(f32)).astype(bf16)

    dn_nt = (((1,), (1,)), ((), ()))

    def g_body(d, _):
        pr, pi = powtab(d, 0, 7, S)
        ar, ai = powtab(d, 14, 19, 32)
        ar, ai = _cmul(ar, ai, pw_s[24, pl.ds(d, 1), :], pw_s[25, pl.ds(d, 1), :])
        lhs = jnp.concatenate([ar[:24], -ai[:24]], axis=1)
        rhs = jnp.concatenate([pr, pi], axis=1)
        lh, ll = split(lhs)
        rh = rhs.astype(bf16)
        g = lax.dot_general(jnp.concatenate([lh, ll], axis=0), rh, dn_nt,
                            preferred_element_type=f32)
        g_s[d] = g[:24] + g[24:]
        return 0

    lax.fori_loop(0, D, g_body, 0, unroll=8)

    for r in range(C + 1):
        gt_s[r] = g_s[:, r, :].T

    for c in range(C):
        uf_s[c] = jnp.dot(fwd_ref[...], xn_s[pl.ds(c * S, S), :], preferred_element_type=f32)
        kf = jnp.dot(fwdk_ref[c], gt_s[c].astype(bf16), preferred_element_type=f32)
        kf_s[c] = kf + xcol_ref[c] * gt_s[c + 1, pl.ds(0, 1), :]

    rb = 16
    nrb = S // rb

    def mac_body(i, _):
        cs = pl.ds(pl.multiple_of((i // nrb) * 128, 128), 128)
        r0 = pl.multiple_of((i % nrb) * rb, rb)
        for t1 in range(C):
            yr = jnp.zeros((rb, 128), f32)
            yi = jnp.zeros((rb, 128), f32)
            for j in range(t1 + 1):
                ur = uf_s[t1 - j, pl.ds(r0, rb), cs]
                ui = uf_s[t1 - j, pl.ds(S + r0, rb), cs]
                kr = kf_s[j, pl.ds(r0, rb), cs]
                ki = kf_s[j, pl.ds(S + r0, rb), cs]
                yr = yr + (ur * kr - ui * ki)
                yi = yi + (ur * ki + ui * kr)
            yf_s[t1, pl.ds(r0, rb), cs] = yr.astype(bf16)
            yf_s[t1, pl.ds(S + r0, rb), cs] = yi.astype(bf16)
        return 0

    lax.fori_loop(0, (D // 128) * nrb, mac_body, 0)

    for c in range(C):
        o = jnp.dot(inv_ref[...], yf_s[c], preferred_element_type=f32)
        if c == 0:
            yacc_s[0] = o[:S]
        else:
            yacc_s[c] = yacc_s[c] + o[:S]
        yacc_s[c + 1] = o[S:]

    w1_copy.wait()
    w2_copy.wait()

    def mlp_body(i, _):
        r0 = pl.multiple_of(i * TB, TB)
        h = jnp.dot(y2_s[pl.ds(r0, TB), :], w1_s[...], preferred_element_type=f32)
        h = h + b1_ref[...].astype(f32)
        gl = _gelu_tanh(h).astype(bf16)
        mlp = jnp.dot(gl, w2_s[...], preferred_element_type=f32) + b2_ref[...].astype(f32)
        nb = TB // S
        yc = jnp.concatenate([yacc_s[i * nb + k] for k in range(nb)], axis=0)
        xn = xn_s[pl.ds(r0, TB), :].astype(f32)
        a_branch = yc.astype(bf16).astype(f32) + xn * dsk_ref[...].astype(f32)
        out = x_ref[pl.ds(r0, TB), :].astype(f32) + a_branch + mlp
        o_ref[pl.ds(r0, TB), :] = out.astype(o_ref.dtype)
        return 0

    lax.fori_loop(0, L // TB, mlp_body, 0)


@jax.jit
def pallas_parallel_sum__ssm_conv_s4__mixer_channel_mlp__prompt_kernel(
    A_u: jax.Array,
    A_A_re: jax.Array,
    A_A_im: jax.Array,
    A_B_re: jax.Array,
    A_B_im: jax.Array,
    A_C_re: jax.Array,
    A_C_im: jax.Array,
    A_log_dt: jax.Array,
    A_Dskip: jax.Array,
    B_x: jax.Array,
    B_w1: jax.Array,
    B_b1: jax.Array,
    B_w2: jax.Array,
    B_b2: jax.Array,
):
    del B_x
    Bsz, L, D = A_u.shape
    assert Bsz == 1
    N = A_A_re.shape[1]
    F = B_w1.shape[1]
    S = _S
    C = L // S
    TB = 256
    fwd_t, fwdk_t, xcol, inv = _const_tables(L)
    bf16 = jnp.bfloat16
    consts = (
        jnp.asarray(fwd_t, bf16),
        jnp.asarray(fwdk_t, bf16),
        jnp.asarray(xcol, jnp.float32),
        jnp.asarray(inv, bf16),
    )
    f32 = jnp.float32
    scratch = [
        pltpu.VMEM((L, D), bf16),
        pltpu.VMEM((L, D), bf16),
        pltpu.VMEM((26, D, N), f32),
        pltpu.VMEM((D, 24, S), f32),
        pltpu.VMEM((C + 1, S, D), f32),
        pltpu.VMEM((C, 2 * S, D), f32),
        pltpu.VMEM((C, 2 * S, D), f32),
        pltpu.VMEM((C, 2 * S, D), bf16),
        pltpu.VMEM((C + 1, S, D), f32),
        pltpu.VMEM((D, F), bf16),
        pltpu.VMEM((F, D), bf16),
        pltpu.SemaphoreType.DMA((2,)),
    ]
    vmem = pl.BlockSpec(memory_space=pltpu.VMEM)
    hbm = pl.BlockSpec(memory_space=pl.ANY)
    in_specs = [vmem] * 9 + [hbm, vmem, hbm, vmem] + [vmem] * 4
    out = pl.pallas_call(
        functools.partial(_kernel, L=L, D=D, N=N, F=F, TB=TB),
        out_shape=jax.ShapeDtypeStruct((L, D), A_u.dtype),
        in_specs=in_specs,
        out_specs=vmem,
        scratch_shapes=scratch,
        compiler_params=pltpu.CompilerParams(vmem_limit_bytes=110 * 1024 * 1024),
    )(
        A_u.reshape(L, D),
        A_A_re, A_A_im, A_B_re, A_B_im, A_C_re, A_C_im,
        A_log_dt.reshape(D, 1),
        A_Dskip.reshape(1, D),
        B_w1, B_b1.reshape(1, F), B_w2, B_b2.reshape(1, D),
        *consts,
    )
    return out.reshape(Bsz, L, D)
```

```python
import functools
import math

import jax
import jax.numpy as jnp
import numpy as np
from jax import lax
import jax.experimental.pallas as pl
import jax.experimental.pallas.tpu as pltpu

_S = 128


def _bf16_round_np(x):
    u = np.asarray(x, np.float32).view(np.uint32).astype(np.uint64)
    u = (u + 0x7FFF + ((u >> 16) & 1)) & 0xFFFF0000
    return u.astype(np.uint32).view(np.float32)


@functools.lru_cache(maxsize=None)
def _const_tables(L):
    S = _S
    C = L // S
    n = np.arange(S)
    b = np.arange(S)
    ang = np.pi * (2 * b[:, None] + 1) * n[None, :] / (2 * S)
    fwd_t = np.concatenate([np.cos(ang), -np.sin(ang)], axis=0)
    q = _bf16_round_np(np.arange(L)).astype(np.int64)
    fwdk_t = np.zeros((C, 2 * S, S))
    xcol = np.zeros((2 * S, C))
    for j in range(C):
        for i in range(S):
            src = q[S * j + i] - S * j
            if src < S:
                fwdk_t[j, :, src] += fwd_t[:, i]
            else:
                assert src == S
                xcol[:, j] += fwd_t[:, i]
    n2 = np.arange(2 * S)
    ang2 = np.pi * (2 * b[None, :] + 1) * n2[:, None] / (2 * S)
    inv = np.concatenate([np.cos(ang2) / S, -np.sin(ang2) / S], axis=1)
    return fwd_t, fwdk_t, xcol, inv


def _cmul(ar, ai, br, bi):
    return ar * br - ai * bi, ar * bi + ai * br


def _gelu_tanh(h):
    c = math.sqrt(2.0 / math.pi)
    return 0.5 * h * (1.0 + jnp.tanh(c * (h + 0.044715 * (h * h * h))))


def _kernel(x_ref, are_ref, aim_ref, bre_ref, bim_ref, cre_ref, cim_ref, ldt_ref, dsk_ref,
            w1_ref, b1_ref, w2_ref, b2_ref, fwd_ref, fwdk_ref, xcol_ref, inv_ref,
            o_ref,
            x_s, xn_s, y2_s, pw_s, g_s, gt_s, uf_s, kf_s, yf_s, yacc_s, w1_s, w2_s, fwdk_s,
            mlp_s, ob_s, sem, osem,
            *, L, D, N, F, TB):
    S = _S
    C = L // S
    f32 = jnp.float32
    bf16 = jnp.bfloat16

    x_copy = pltpu.make_async_copy(x_ref, x_s, sem.at[0])
    fk_copy = pltpu.make_async_copy(fwdk_ref, fwdk_s, sem.at[1])
    w1_copy = pltpu.make_async_copy(w1_ref, w1_s, sem.at[2])
    w2_copy = pltpu.make_async_copy(w2_ref, w2_s, sem.at[3])
    x_copy.start()
    fk_copy.start()
    w1_copy.start()
    w2_copy.start()

    def ln(v):
        m = jnp.mean(v, axis=-1, keepdims=True)
        c = v - m
        var = jnp.mean(c * c, axis=-1, keepdims=True)
        return c * lax.rsqrt(var + 1e-5)

    def ln_body(i, _):
        r0 = pl.multiple_of(i * TB, TB)
        xv = x_s[pl.ds(r0, TB), :].astype(f32)
        xn = ln(xv).astype(bf16)
        xn_s[pl.ds(r0, TB), :] = xn
        y2_s[pl.ds(r0, TB), :] = ln(xn.astype(f32)).astype(bf16)
        return 0

    dt = jnp.exp(ldt_ref[...].astype(f32)).astype(bf16).astype(f32)
    lr = dt * are_ref[...].astype(f32)
    li = dt * aim_ref[...].astype(f32)
    mag = jnp.exp(lr)
    zr, zi = mag * jnp.cos(li), mag * jnp.sin(li)
    for k in range(7):
        pw_s[k] = zr
        pw_s[7 + k] = zi
        if k < 6:
            zr, zi = _cmul(zr, zi, zr, zi)
    mag = jnp.exp(lr * float(S))
    er, ei = mag * jnp.cos(li * float(S)), mag * jnp.sin(li * float(S))
    for k in range(5):
        pw_s[14 + k] = er
        pw_s[19 + k] = ei
        if k < 4:
            er, ei = _cmul(er, ei, er, ei)
    cbr, cbi = _cmul(cre_ref[...].astype(f32), cim_ref[...].astype(f32),
                     dt * bre_ref[...].astype(f32), dt * bim_ref[...].astype(f32))
    pw_s[24] = cbr
    pw_s[25] = cbi

    sub = lax.broadcasted_iota(jnp.int32, (8, N), 0)
    one = jnp.ones((8, N), f32)
    zero = jnp.zeros((8, N), f32)

    def powtab(d, rbase, ibase, nrows):
        def row(k, base):
            return pw_s[base + k, pl.ds(d, 1), :]
        pr = jnp.where((sub & 1) == 1, row(0, rbase), one)
        pi = jnp.where((sub & 1) == 1, row(0, ibase), zero)
        for k in (1, 2):
            tr = jnp.where((sub & (1 << k)) != 0, row(k, rbase), one)
            ti = jnp.where((sub & (1 << k)) != 0, row(k, ibase), zero)
            pr, pi = _cmul(pr, pi, tr, ti)
        k = 3
        n = 8
        while n < nrows:
            qr, qi = _cmul(pr, pi, row(k, rbase), row(k, ibase))
            pr = jnp.concatenate([pr, qr], axis=0)
            pi = jnp.concatenate([pi, qi], axis=0)
            n *= 2
            k += 1
        return pr, pi

    def split(v):
        h = v.astype(bf16)
        return h, (v - h.astype(f32)).astype(bf16)

    dn_nt = (((1,), (1,)), ((), ()))

    def g_body(d, _):
        pr, pi = powtab(d, 0, 7, S)
        ar, ai = powtab(d, 14, 19, 32)
        ar, ai = _cmul(ar, ai, pw_s[24, pl.ds(d, 1), :], pw_s[25, pl.ds(d, 1), :])
        lhs = jnp.concatenate([ar[:24], -ai[:24]], axis=1)
        rhs = jnp.concatenate([pr, pi], axis=1)
        lh, ll = split(lhs)
        rh = rhs.astype(bf16)
        g = lax.dot_general(jnp.concatenate([lh, ll], axis=0), rh, dn_nt,
                            preferred_element_type=f32)
        g_s[d] = g[:24] + g[24:]
        return 0

    lax.fori_loop(0, D, g_body, 0, unroll=8)

    for r in range(C + 1):
        gt_s[r] = g_s[:, r, :].T

    x_copy.wait()
    lax.fori_loop(0, L // TB, ln_body, 0)

    fk_copy.wait()
    for c in range(C):
        uf_s[c] = jnp.dot(fwd_ref[...], xn_s[pl.ds(c * S, S), :], preferred_element_type=f32)
        kf = jnp.dot(fwdk_s[c], gt_s[c].astype(bf16), preferred_element_type=f32)
        kf_s[c] = kf + xcol_ref[:, pl.ds(c, 1)] * gt_s[c + 1, pl.ds(0, 1), :]

    rb = 16
    nrb = S // rb
    nblk = L // TB
    nmac = (D // 128) * nrb // nblk

    def mac_block(i):
        cs = pl.ds(pl.multiple_of((i // nrb) * 128, 128), 128)
        r0 = pl.multiple_of((i % nrb) * rb, rb)
        for t1 in range(C):
            yr = jnp.zeros((rb, 128), f32)
            yi = jnp.zeros((rb, 128), f32)
            for j in range(t1 + 1):
                ur = uf_s[t1 - j, pl.ds(r0, rb), cs]
                ui = uf_s[t1 - j, pl.ds(S + r0, rb), cs]
                kr = kf_s[j, pl.ds(r0, rb), cs]
                ki = kf_s[j, pl.ds(S + r0, rb), cs]
                yr = yr + (ur * kr - ui * ki)
                yi = yi + (ur * ki + ui * kr)
            yf_s[t1, pl.ds(r0, rb), cs] = yr.astype(bf16)
            yf_s[t1, pl.ds(S + r0, rb), cs] = yi.astype(bf16)

    w1_copy.wait()
    w2_copy.wait()

    def df_body(i, _):
        r0 = pl.multiple_of(i * TB, TB)
        h = jnp.dot(y2_s[pl.ds(r0, TB), :], w1_s[...], preferred_element_type=f32)
        h = h + b1_ref[...].astype(f32)
        gl = _gelu_tanh(h).astype(bf16)
        mlp = jnp.dot(gl, w2_s[...], preferred_element_type=f32) + b2_ref[...].astype(f32)
        mlp_s[pl.ds(r0, TB), :] = mlp
        for k in range(nmac):
            mac_block(i * nmac + k)
        return 0

    lax.fori_loop(0, nblk, df_body, 0)

    for c in range(C):
        o = jnp.dot(inv_ref[...], yf_s[c], preferred_element_type=f32)
        if c == 0:
            yacc_s[0] = o[:S]
        else:
            yacc_s[c] = yacc_s[c] + o[:S]
        yacc_s[c + 1] = o[S:]

    nb = TB // S
    out_copies = []
    for i in range(nblk):
        r0 = i * TB
        yc = jnp.concatenate([yacc_s[i * nb + k] for k in range(nb)], axis=0)
        xn = xn_s[pl.ds(r0, TB), :].astype(f32)
        a_branch = yc.astype(bf16).astype(f32) + xn * dsk_ref[...].astype(f32)
        out = x_s[pl.ds(r0, TB), :].astype(f32) + a_branch + mlp_s[pl.ds(r0, TB), :]
        ob_s[pl.ds(r0, TB), :] = out.astype(ob_s.dtype)
        cp = pltpu.make_async_copy(ob_s.at[pl.ds(r0, TB), :], o_ref.at[pl.ds(r0, TB), :],
                                   osem.at[i])
        cp.start()
        out_copies.append(cp)
    for cp in out_copies:
        cp.wait()


@jax.jit
def pallas_parallel_sum__ssm_conv_s4__mixer_channel_mlp__prompt_kernel(
    A_u: jax.Array,
    A_A_re: jax.Array,
    A_A_im: jax.Array,
    A_B_re: jax.Array,
    A_B_im: jax.Array,
    A_C_re: jax.Array,
    A_C_im: jax.Array,
    A_log_dt: jax.Array,
    A_Dskip: jax.Array,
    B_x: jax.Array,
    B_w1: jax.Array,
    B_b1: jax.Array,
    B_w2: jax.Array,
    B_b2: jax.Array,
):
    del B_x
    Bsz, L, D = A_u.shape
    assert Bsz == 1
    N = A_A_re.shape[1]
    F = B_w1.shape[1]
    S = _S
    C = L // S
    TB = 256
    fwd_t, fwdk_t, xcol, inv = _const_tables(L)
    bf16 = jnp.bfloat16
    consts = (
        jnp.asarray(fwd_t, bf16),
        jnp.asarray(fwdk_t, bf16),
        jnp.asarray(xcol, jnp.float32),
        jnp.asarray(inv, bf16),
    )
    f32 = jnp.float32
    scratch = [
        pltpu.VMEM((L, D), bf16),
        pltpu.VMEM((L, D), bf16),
        pltpu.VMEM((L, D), bf16),
        pltpu.VMEM((26, D, N), f32),
        pltpu.VMEM((D, 24, S), f32),
        pltpu.VMEM((C + 1, S, D), f32),
        pltpu.VMEM((C, 2 * S, D), f32),
        pltpu.VMEM((C, 2 * S, D), f32),
        pltpu.VMEM((C, 2 * S, D), bf16),
        pltpu.VMEM((C + 1, S, D), f32),
        pltpu.VMEM((D, F), bf16),
        pltpu.VMEM((F, D), bf16),
        pltpu.VMEM((C, 2 * S, S), bf16),
        pltpu.VMEM((L, D), f32),
        pltpu.VMEM((L, D), A_u.dtype),
        pltpu.SemaphoreType.DMA((4,)),
        pltpu.SemaphoreType.DMA((L // TB,)),
    ]
    vmem = pl.BlockSpec(memory_space=pltpu.VMEM)
    hbm = pl.BlockSpec(memory_space=pl.ANY)
    in_specs = [hbm] + [vmem] * 8 + [hbm, vmem, hbm, vmem] + [vmem, hbm, vmem, vmem]
    out = pl.pallas_call(
        functools.partial(_kernel, L=L, D=D, N=N, F=F, TB=TB),
        out_shape=jax.ShapeDtypeStruct((L, D), A_u.dtype),
        in_specs=in_specs,
        out_specs=hbm,
        scratch_shapes=scratch,
        compiler_params=pltpu.CompilerParams(vmem_limit_bytes=110 * 1024 * 1024),
    )(
        A_u.reshape(L, D),
        A_A_re, A_A_im, A_B_re, A_B_im, A_C_re, A_C_im,
        A_log_dt.reshape(D, 1),
        A_Dskip.reshape(1, D),
        B_w1, B_b1.reshape(1, F), B_w2, B_b2.reshape(1, D),
        *consts,
    )
    return out.reshape(Bsz, L, D)
```

```python
import functools
import math

import jax
import jax.numpy as jnp
import numpy as np
from jax import lax
import jax.experimental.pallas as pl
import jax.experimental.pallas.tpu as pltpu

_S = 128


def _bf16_round_np(x):
    u = np.asarray(x, np.float32).view(np.uint32).astype(np.uint64)
    u = (u + 0x7FFF + ((u >> 16) & 1)) & 0xFFFF0000
    return u.astype(np.uint32).view(np.float32)


@functools.lru_cache(maxsize=None)
def _const_tables(L):
    S = _S
    C = L // S
    n = np.arange(S)
    b = np.arange(S)
    ang = np.pi * (2 * b[:, None] + 1) * n[None, :] / (2 * S)
    fwd_t = np.concatenate([np.cos(ang), -np.sin(ang)], axis=0)
    q = _bf16_round_np(np.arange(L)).astype(np.int64)
    fwdk_t = np.zeros((C, 2 * S, S))
    xcol = np.zeros((2 * S, C))
    for j in range(C):
        for i in range(S):
            src = q[S * j + i] - S * j
            if src < S:
                fwdk_t[j, :, src] += fwd_t[:, i]
            else:
                assert src == S
                xcol[:, j] += fwd_t[:, i]
    n2 = np.arange(2 * S)
    ang2 = np.pi * (2 * b[None, :] + 1) * n2[:, None] / (2 * S)
    inv = np.concatenate([np.cos(ang2) / S, -np.sin(ang2) / S], axis=1)
    return fwd_t, fwdk_t, xcol, inv


def _cmul(ar, ai, br, bi):
    return ar * br - ai * bi, ar * bi + ai * br


def _gelu_tanh(h):
    c = math.sqrt(2.0 / math.pi)
    return 0.5 * h * (1.0 + jnp.tanh(c * (h + 0.044715 * (h * h * h))))


def _kernel(x_ref, are_ref, aim_ref, bre_ref, bim_ref, cre_ref, cim_ref, ldt_ref, dsk_ref,
            w1_ref, b1_ref, w2_ref, b2_ref, fwd_ref, fwdk_ref, xcol_ref, inv_ref,
            o_ref,
            x_s, xn_s, y2_s, pw_s, g_s, gt_s, uf_s, kf_s, yf_s, yacc_s, w1_s, w2_s, fwdk_s,
            mlp_s, ob_s, sem, osem,
            *, L, D, N, F, TB):
    S = _S
    C = L // S
    f32 = jnp.float32
    bf16 = jnp.bfloat16

    x_copy = pltpu.make_async_copy(x_ref, x_s, sem.at[0])
    fk_copy = pltpu.make_async_copy(fwdk_ref, fwdk_s, sem.at[1])
    w1_copy = pltpu.make_async_copy(w1_ref, w1_s, sem.at[2])
    w2_copy = pltpu.make_async_copy(w2_ref, w2_s, sem.at[3])
    x_copy.start()
    fk_copy.start()
    w1_copy.start()
    w2_copy.start()

    def ln(v):
        m = jnp.mean(v, axis=-1, keepdims=True)
        c = v - m
        var = jnp.mean(c * c, axis=-1, keepdims=True)
        return c * lax.rsqrt(var + 1e-5)

    def ln_body(i, _):
        r0 = pl.multiple_of(i * TB, TB)
        xv = x_s[pl.ds(r0, TB), :].astype(f32)
        xn = ln(xv).astype(bf16)
        xn_s[pl.ds(r0, TB), :] = xn
        y2_s[pl.ds(r0, TB), :] = ln(xn.astype(f32)).astype(bf16)
        return 0

    dt = jnp.exp(ldt_ref[...].astype(f32)).astype(bf16).astype(f32)
    lr = dt * are_ref[...].astype(f32)
    li = dt * aim_ref[...].astype(f32)
    mag = jnp.exp(lr)
    zr, zi = mag * jnp.cos(li), mag * jnp.sin(li)
    for k in range(7):
        pw_s[k] = zr
        pw_s[7 + k] = zi
        if k < 6:
            zr, zi = _cmul(zr, zi, zr, zi)
    mag = jnp.exp(lr * float(S))
    er, ei = mag * jnp.cos(li * float(S)), mag * jnp.sin(li * float(S))
    for k in range(5):
        pw_s[14 + k] = er
        pw_s[19 + k] = ei
        if k < 4:
            er, ei = _cmul(er, ei, er, ei)
    cbr, cbi = _cmul(cre_ref[...].astype(f32), cim_ref[...].astype(f32),
                     dt * bre_ref[...].astype(f32), dt * bim_ref[...].astype(f32))
    pw_s[24] = cbr
    pw_s[25] = cbi

    sub = lax.broadcasted_iota(jnp.int32, (8, N), 0)
    one = jnp.ones((8, N), f32)
    zero = jnp.zeros((8, N), f32)

    def powtab(d, rbase, ibase, nrows):
        def row(k, base):
            return pw_s[base + k, pl.ds(d, 1), :]
        pr = jnp.where((sub & 1) == 1, row(0, rbase), one)
        pi = jnp.where((sub & 1) == 1, row(0, ibase), zero)
        for k in (1, 2):
            tr = jnp.where((sub & (1 << k)) != 0, row(k, rbase), one)
            ti = jnp.where((sub & (1 << k)) != 0, row(k, ibase), zero)
            pr, pi = _cmul(pr, pi, tr, ti)
        k = 3
        n = 8
        while n < nrows:
            qr, qi = _cmul(pr, pi, row(k, rbase), row(k, ibase))
            pr = jnp.concatenate([pr, qr], axis=0)
            pi = jnp.concatenate([pi, qi], axis=0)
            n *= 2
            k += 1
        return pr, pi

    def split(v):
        h = v.astype(bf16)
        return h, (v - h.astype(f32)).astype(bf16)

    dn_nt = (((1,), (1,)), ((), ()))

    def g_body(d, _):
        pr, pi = powtab(d, 0, 7, S)
        ar, ai = powtab(d, 14, 19, 32)
        ar, ai = _cmul(ar, ai, pw_s[24, pl.ds(d, 1), :], pw_s[25, pl.ds(d, 1), :])
        lhs = jnp.concatenate([ar[:24], -ai[:24]], axis=1)
        rhs = jnp.concatenate([pr, pi], axis=1)
        lh, ll = split(lhs)
        rh = rhs.astype(bf16)
        g = lax.dot_general(jnp.concatenate([lh, ll], axis=0), rh, dn_nt,
                            preferred_element_type=f32)
        g_s[d] = g[:24] + g[24:]
        return 0

    x_copy.wait()
    lax.fori_loop(0, L // TB, ln_body, 0)
    w1_copy.wait()
    w2_copy.wait()
    TM = 256
    nit = L // TM
    chp = D // nit

    def bm_body(i, _):
        r0 = pl.multiple_of(i * TM, TM)
        h = jnp.dot(y2_s[pl.ds(r0, TM), :], w1_s[...], preferred_element_type=f32)
        h = h + b1_ref[...].astype(f32)
        gl = _gelu_tanh(h).astype(bf16)
        mlp = jnp.dot(gl, w2_s[...], preferred_element_type=f32) + b2_ref[...].astype(f32)
        mlp_s[pl.ds(r0, TM), :] = mlp
        for k in range(chp):
            g_body(i * chp + k, 0)
        return 0

    lax.fori_loop(0, nit, bm_body, 0)

    for r in range(C + 1):
        gt_s[r] = g_s[:, r, :].T

    fk_copy.wait()
    for c in range(C):
        uf_s[c] = jnp.dot(fwd_ref[...], xn_s[pl.ds(c * S, S), :], preferred_element_type=f32)
        kf = jnp.dot(fwdk_s[c], gt_s[c].astype(bf16), preferred_element_type=f32)
        kf_s[c] = kf + xcol_ref[:, pl.ds(c, 1)] * gt_s[c + 1, pl.ds(0, 1), :]

    rb = 16
    nrb = S // rb
    nblk = L // TB
    nmac = (D // 128) * nrb // nblk

    def mac_block(i):
        cs = pl.ds(pl.multiple_of((i // nrb) * 128, 128), 128)
        r0 = pl.multiple_of((i % nrb) * rb, rb)
        for t1 in range(C):
            yr = jnp.zeros((rb, 128), f32)
            yi = jnp.zeros((rb, 128), f32)
            for j in range(t1 + 1):
                ur = uf_s[t1 - j, pl.ds(r0, rb), cs]
                ui = uf_s[t1 - j, pl.ds(S + r0, rb), cs]
                kr = kf_s[j, pl.ds(r0, rb), cs]
                ki = kf_s[j, pl.ds(S + r0, rb), cs]
                yr = yr + (ur * kr - ui * ki)
                yi = yi + (ur * ki + ui * kr)
            yf_s[t1, pl.ds(r0, rb), cs] = yr.astype(bf16)
            yf_s[t1, pl.ds(S + r0, rb), cs] = yi.astype(bf16)

    def df_body(i, _):
        for k in range(nmac):
            mac_block(i * nmac + k)
        return 0

    lax.fori_loop(0, nblk, df_body, 0)

    for c in range(C):
        o = jnp.dot(inv_ref[...], yf_s[c], preferred_element_type=f32)
        if c == 0:
            yacc_s[0] = o[:S]
        else:
            yacc_s[c] = yacc_s[c] + o[:S]
        yacc_s[c + 1] = o[S:]

    nb = TB // S
    out_copies = []
    for i in range(nblk):
        r0 = i * TB
        yc = jnp.concatenate([yacc_s[i * nb + k] for k in range(nb)], axis=0)
        xn = xn_s[pl.ds(r0, TB), :].astype(f32)
        a_branch = yc.astype(bf16).astype(f32) + xn * dsk_ref[...].astype(f32)
        out = x_s[pl.ds(r0, TB), :].astype(f32) + a_branch + mlp_s[pl.ds(r0, TB), :]
        ob_s[pl.ds(r0, TB), :] = out.astype(ob_s.dtype)
        cp = pltpu.make_async_copy(ob_s.at[pl.ds(r0, TB), :], o_ref.at[pl.ds(r0, TB), :],
                                   osem.at[i])
        cp.start()
        out_copies.append(cp)
    for cp in out_copies:
        cp.wait()


@jax.jit
def pallas_parallel_sum__ssm_conv_s4__mixer_channel_mlp__prompt_kernel(
    A_u: jax.Array,
    A_A_re: jax.Array,
    A_A_im: jax.Array,
    A_B_re: jax.Array,
    A_B_im: jax.Array,
    A_C_re: jax.Array,
    A_C_im: jax.Array,
    A_log_dt: jax.Array,
    A_Dskip: jax.Array,
    B_x: jax.Array,
    B_w1: jax.Array,
    B_b1: jax.Array,
    B_w2: jax.Array,
    B_b2: jax.Array,
):
    del B_x
    Bsz, L, D = A_u.shape
    assert Bsz == 1
    N = A_A_re.shape[1]
    F = B_w1.shape[1]
    S = _S
    C = L // S
    TB = 256
    fwd_t, fwdk_t, xcol, inv = _const_tables(L)
    bf16 = jnp.bfloat16
    consts = (
        jnp.asarray(fwd_t, bf16),
        jnp.asarray(fwdk_t, bf16),
        jnp.asarray(xcol, jnp.float32),
        jnp.asarray(inv, bf16),
    )
    f32 = jnp.float32
    scratch = [
        pltpu.VMEM((L, D), bf16),
        pltpu.VMEM((L, D), bf16),
        pltpu.VMEM((L, D), bf16),
        pltpu.VMEM((26, D, N), f32),
        pltpu.VMEM((D, 24, S), f32),
        pltpu.VMEM((C + 1, S, D), f32),
        pltpu.VMEM((C, 2 * S, D), f32),
        pltpu.VMEM((C, 2 * S, D), f32),
        pltpu.VMEM((C, 2 * S, D), bf16),
        pltpu.VMEM((C + 1, S, D), f32),
        pltpu.VMEM((D, F), bf16),
        pltpu.VMEM((F, D), bf16),
        pltpu.VMEM((C, 2 * S, S), bf16),
        pltpu.VMEM((L, D), f32),
        pltpu.VMEM((L, D), A_u.dtype),
        pltpu.SemaphoreType.DMA((4,)),
        pltpu.SemaphoreType.DMA((L // TB,)),
    ]
    vmem = pl.BlockSpec(memory_space=pltpu.VMEM)
    hbm = pl.BlockSpec(memory_space=pl.ANY)
    in_specs = [hbm] + [vmem] * 8 + [hbm, vmem, hbm, vmem] + [vmem, hbm, vmem, vmem]
    out = pl.pallas_call(
        functools.partial(_kernel, L=L, D=D, N=N, F=F, TB=TB),
        out_shape=jax.ShapeDtypeStruct((L, D), A_u.dtype),
        in_specs=in_specs,
        out_specs=hbm,
        scratch_shapes=scratch,
        compiler_params=pltpu.CompilerParams(vmem_limit_bytes=110 * 1024 * 1024),
    )(
        A_u.reshape(L, D),
        A_A_re, A_A_im, A_B_re, A_B_im, A_C_re, A_C_im,
        A_log_dt.reshape(D, 1),
        A_Dskip.reshape(1, D),
        B_w1, B_b1.reshape(1, F), B_w2, B_b2.reshape(1, D),
        *consts,
    )
    return out.reshape(Bsz, L, D)
```
